```python
import os as _os
_os.environ.setdefault("JAX_PLATFORMS", "cpu")
import jax
import jax.numpy as jnp

def _softmax(x, axis=-1):
    return jax.nn.softmax(x, axis=axis)
def _gelu(x):
    return jax.nn.gelu(x, approximate=True)
def _silu(x):
    return jax.nn.silu(x)
def _sigmoid(x):
    return jax.nn.sigmoid(x)
def _layernorm(x, axis=-1, eps=1e-5):
    m = jnp.mean(x, axis=axis, keepdims=True)
    v = jnp.var(x, axis=axis, keepdims=True)
    return (x - m) / jnp.sqrt(v + eps)
def _scatter_add(tgt, idx, src, axis=0):
    return tgt.at[idx].add(src)
def _segment_sum(src, seg, n):
    return jax.ops.segment_sum(src, seg, n)
class _Rng:
    def __init__(self, key):
        self._k = key
    def _next(self):
        self._k, sub = jax.random.split(self._k)
        return sub
    def normal(self, shape):
        return jax.random.normal(self._next(), shape, dtype=jnp.bfloat16)
    def randint(self, lo, hi, shape):
        return jax.random.randint(self._next(), shape, lo, hi, dtype=jnp.int32)
    def uniform(self, shape, lo=0.0, hi=1.0):
        return jax.random.uniform(self._next(), shape, jnp.bfloat16, lo, hi)
    def permutation(self, n):
        return jax.random.permutation(self._next(), n)


kernel_name = 'sequential_preLN__sliding_local_dilated__dense_activation_relu__prompt'

def setup_inputs():
    _rng = _Rng(jax.random.key(int.from_bytes(__import__("os").urandom(4), "little")))
    _w = (lambda a: (lambda t: t.astype(jnp.bfloat16) if jnp.issubdtype(t.dtype, jnp.floating) else t)(jnp.asarray(a)))
    def _A_setup():
        B, S, D = 1, 2048, 1024
        return {
            "x": _w((lambda *s: _rng.normal(s) * 0.05)(B, S, D)),
            "wqkv": _w((lambda *s: _rng.normal(s) * 0.05)(D, 3 * D)),
            "wo": _w((lambda *s: _rng.normal(s) * 0.05)(D, D)),
        }
    _A_in = _A_setup()

    def _B_setup():
        B, S, D, Dff = 1, 2048, 1024, 3584
        return {
            "x": _w((lambda *s: _rng.normal(s) * 0.05)(B, S, D)),
            "w1": _w((lambda *s: _rng.normal(s) * 0.05)(D, Dff)),
            "w2": _w((lambda *s: _rng.normal(s) * 0.05)(Dff, D)),
        }
    _B_in = _B_setup()

    return {
        "A_x": _A_in["x"],
        "A_wqkv": _A_in["wqkv"],
        "A_wo": _A_in["wo"],
        "B_x": _B_in["x"],
        "B_w1": _B_in["w1"],
        "B_w2": _B_in["w2"],
    }

def reference(A_x, A_wqkv, A_wo, B_x, B_w1, B_w2):
    def _A_ref(x, wqkv, wo):
        B, S, D = x.shape
        H = 32; Dh = D // H
        W, dil = 8, 2
        qkv = (lambda x, *d: x.transpose(*d))((x @ wqkv).reshape(B, S, 3, H, Dh), 2, 0, 3, 1, 4)
        q, k, v = qkv[0], qkv[1], qkv[2]
        scale = Dh ** -0.5
        pos = jnp.arange(S)
        off = jnp.arange(W) * dil
        idx = pos[:, None] - off[None, :]
        mask = idx >= 0
        idx_c = jnp.where(mask, idx, 0).reshape(-1)
        kg = k[:, :, idx_c, :].reshape(B, H, S, W, Dh)
        vg = v[:, :, idx_c, :].reshape(B, H, S, W, Dh)
        logits = jnp.einsum("bhsd,bhswd->bhsw", q, kg) * scale
        logits = jnp.where(mask[None, None, :, :], logits, -1e9)
        attn = _softmax(logits, axis=-1)
        o = jnp.einsum("bhsw,bhswd->bhsd", attn, vg)
        return (lambda x, *d: x.transpose(*d))(o, 0, 2, 1, 3).reshape(B, S, D) @ wo

    def _B_ref(x, w1, w2):
        h = jnp.einsum("bsd,df->bsf", x, w1)
        zero = jnp.zeros_like(h)
        h = jnp.maximum(h, zero)
        return jnp.einsum("bsf,fd->bsd", h, w2)

    x = A_x
    h = x + _A_ref(_layernorm(x, axis=-1), A_wqkv, A_wo)
    h2 = h + _B_ref(_layernorm(h, axis=-1), B_w1, B_w2)
    return h2
```

```python
import functools
import jax, jax.numpy as jnp
import jax.experimental.pallas as pl
import jax.experimental.pallas.tpu as pltpu

S, D, DFF, H, DH, W = 2048, 1024, 3584, 32, 32, 8
HALO = 16
F32, BF16, U32, I32 = jnp.float32, jnp.bfloat16, jnp.uint32, jnp.int32
NT = D // 128

def _ln(x):
    m = jnp.mean(x, axis=-1, keepdims=True)
    xc = x - m
    v = jnp.mean(xc * xc, axis=-1, keepdims=True)
    return xc * jax.lax.rsqrt(v + 1e-5)

def to_phys(x):
    R, C = x.shape
    return x.reshape(R // 8, 8, C // 128, 128).transpose(0, 2, 1, 3).reshape(R * C // 128, 128)

def dep_of(u):
    t = u[0]
    for a in u[1:]:
        t = t | a
    r = t[0:8]
    for g in range(1, t.shape[0] // 8):
        r = r | t[g*8:(g+1)*8]
    return r

def gate_r(rhs, dep, pred, k0=0):
    if dep is None:
        return rhs
    t = pltpu.bitcast(rhs[k0:k0+16, 0:128], U32)
    t = pltpu.bitcast(jnp.where(pred, t, dep), BF16)
    if rhs.shape[1] > 128:
        t = jnp.concatenate([t, rhs[k0:k0+16, 128:]], axis=1)
    parts = ([rhs[0:k0]] if k0 else []) + [t, rhs[k0+16:, :]]
    return jnp.concatenate(parts, axis=0)

OPT = dict(red=0)
def attn_chunk(i, r0, R, qkv, o_scr, TM):
    scale = DH ** -0.5
    qs = [qkv[j, pl.ds(HALO + r0, R), :] for j in range(NT)]
    ls = []
    for w in range(W):
        s = None
        for j in range(NT):
            p = qs[j] * qkv[NT + j, pl.ds(HALO + r0 - 2 * w, R), :]
            s = p if s is None else s + p
        ls.append(s)
    lane = jax.lax.broadcasted_iota(I32, (R, 128), 1)
    if OPT['red'] == 0:
        ls = [s + jnp.take_along_axis(s, lane ^ 1, axis=1) for s in ls]
        ls = [s + jnp.take_along_axis(s, lane ^ 2, axis=1) for s in ls]
    elif OPT['red'] == 1:
        ls = [s + pltpu.roll(s, 1, 1) for s in ls]
        ls = [s + pltpu.roll(s, 2, 1) for s in ls]
    ls = [s * scale for s in ls]
    for w in range(W):
        if r0 < 2 * w:
            row = jax.lax.broadcasted_iota(jnp.int32, (R, 128), 0) + (r0 + i * TM)
            ls[w] = jnp.where(row >= 2 * w, ls[w], -1e9)
    m = ls[0]
    for w in range(1, W):
        m = jnp.maximum(m, ls[w])
    es = [jnp.exp(l - m) for l in ls]
    den = es[0]
    for w in range(1, W):
        den = den + es[w]
    inv = 1.0 / den
    ps = [e * inv for e in es]
    if OPT['red'] == 1:
        ps = [jnp.where((lane & 1) == 1, p, pltpu.roll(p, 127, 1)) for p in ps]
        ps = [jnp.where((lane & 2) == 2, p, pltpu.roll(p, 126, 1)) for p in ps]
    outs = []
    for j in range(NT):
        o = None
        for w in range(W):
            t = qkv[2 * NT + j, pl.ds(HALO + r0 - 2 * w, R), :] * ps[w]
            o = t if o is None else o + t
        outs.append(o)
    o = jnp.concatenate(outs, axis=1).astype(BF16)
    for j in range(NT):
        o_scr[j, pl.ds(r0, R), :] = o[:, j*128:(j+1)*128]
    u = pltpu.bitcast(o, U32)
    return dep_of([u[:, j*128:(j+1)*128] for j in range(NT)])

def ln_chunk(src, dst_ref, r0, R):
    xn = _ln(src.astype(F32)).astype(BF16)
    u = pltpu.bitcast(xn, U32)
    for j in range(NT):
        dst_ref[j, pl.ds(r0, R), :] = xn[:, j*128:(j+1)*128]
    return dep_of([u[:, j*128:(j+1)*128] for j in range(NT)])

def load_tiles(ref):
    return jnp.concatenate([ref[j] for j in range(NT)], axis=1)

def _or(deps):
    deps = [d for d in deps if d is not None]
    if not deps:
        return None
    r = deps[0]
    for d in deps[1:]:
        r = r | d
    return r

def permute_wqkv_rows(w_scr, r0, nrows, SUB):
    lane = jax.lax.broadcasted_iota(I32, (SUB // 2, 128), 1)
    grp = (lane >> 2) & 7
    masks = [grp == b for b in range(8)]
    units = [(g, s0) for g in range(3) for s0 in range(0, nrows, SUB)]
    def s1(u):
        g, s0 = u
        out = []
        for j in range(NT):
            v = pltpu.bitcast(w_scr[g * NT + j, pl.ds(r0 + s0, SUB), :], I32)
            out.append(pltpu.roll(v, 4 * j, 1) if j else v)
        return out
    def s2(u, rs):
        g, s0 = u
        for t in range(NT):
            o = rs[0]
            for j in range(1, NT):
                o = jnp.where(masks[(t + j) & 7], rs[j], o)
            o = pltpu.roll(o, 128 - 4 * t, 1) if t else o
            w_scr[g * NT + t, pl.ds(r0 + s0, SUB), :] = pltpu.bitcast(o, BF16)
    prev = s1(units[0])
    for n, u in enumerate(units):
        nxt = s1(units[n + 1]) if n + 1 < len(units) else None
        s2(u, prev)
        prev = nxt

def permute_wo(wo_scr, cols):
    sub = jax.lax.broadcasted_iota(I32, (8, 128), 0)
    m4 = (sub & 4) == 0
    m2 = (sub & 2) == 0
    for c in cols:
        for hh in range(4):
            v = {(j, t2): pltpu.bitcast(wo_scr[c, pl.ds(2 * (64 * j + 16 * hh + 8 * t2), 16), :], I32)
                 for j in range(8) for t2 in range(2)}
            for t2 in range(2):
                u = [v[(j, t2)] for j in range(8)]
                for j in (0, 1, 4, 5):
                    a, b = u[j], u[j + 2]
                    u[j] = jnp.where(m4, a, pltpu.roll(b, 4, 0))
                    u[j + 2] = jnp.where(m4, pltpu.roll(a, 4, 0), b)
                for j in (0, 2, 4, 6):
                    a, b = u[j], u[j + 1]
                    u[j] = jnp.where(m2, a, pltpu.roll(b, 2, 0))
                    u[j + 1] = jnp.where(m2, pltpu.roll(a, 6, 0), b)
                for idx in range(8):
                    j2, t1, t0 = idx >> 2, (idx >> 1) & 1, idx & 1
                    t = 4 * t2 + 2 * t1 + t0
                    wo_scr[c, pl.ds(2 * (64 * t + 16 * hh + 8 * j2), 16), :] = pltpu.bitcast(u[idx], BF16)

def _fused(A_x, A_wqkv, A_wo, B_x, B_w1, B_w2, TM=256, R=16, LR=32, NC1=256, KS2=2, NQ=256, FRAC=1.0, S0=1,
          SUB=64, PN=2, W2BAR=1, LRN=32, Q0=1, XS=8, EARLY1=0, NSTEPS=0, flags=None, **opt):
    OPT.update(opt)
    x = A_x.reshape(S, D)
    wo_p = A_wo
    NB = S // TM
    KC = 128
    def kern(x_hbm, wqkv_hbm, wo_hbm, w1_hbm, w2_hbm, o_ref,
             xbuf, wE, wO, wo_ref, w1_ref, w2_ref, sem_x, sem_w, sem_o,
             xn_scr, qkv, o_scr, h_scr, hn_scr):
        i = pl.program_id(0)
        pred = i < 1000
        def cp_x(b):
            return pltpu.make_async_copy(x_hbm.at[pl.ds(pl.multiple_of(b * TM, TM), TM), :], xbuf.at[b % 3], sem_x.at[b % 3])
        def cps_w(m, par):
            dst = wE if par == 0 else wO
            r = pl.multiple_of((2 * m + par) * KC, KC)
            rd = pl.multiple_of(m * KC, KC)
            return [pltpu.make_async_copy(wqkv_hbm.at[pl.ds(r, KC), pl.ds(n * 128, 128)], dst.at[n, pl.ds(rd, KC), :], sem_w.at[2 * m + par])
                    for n in range(3 * NT)]
        def wait_w(m, par):
            dst = wE if par == 0 else wO
            d = dst.at[:, pl.ds(pl.multiple_of(m * KC, KC), KC), :]
            pltpu.make_async_copy(d, d, sem_w.at[2 * m + par]).wait()
        def cps_x0():
            return [pltpu.make_async_copy(x_hbm.at[pl.ds(r, TM // XS), :], xbuf.at[0, pl.ds(r, TM // XS), :], sem_x.at[0]) for r in range(0, TM, TM // XS)]
        def cps_tiles(src, dst, sem):
            return [pltpu.make_async_copy(src.at[:, pl.ds(n * 128, 128)], dst.at[n], sem) for n in range(dst.shape[0])]
        def start(cps):
            for c in cps:
                c.start()
        def wait_all(dst, sem):
            pltpu.make_async_copy(dst, dst, sem).wait()

        def halo():
            for j in range(NT, 3 * NT):
                qkv[j, pl.ds(0, HALO), :] = qkv[j, pl.ds(TM, HALO), :]

        def mxu_chunk(src, m):
            xt = xn_scr_k = None
            return None

        @pl.when(i == 0)
        def _():
            start(cps_w(0, 0))
            start(cps_x0())
            qkv[...] = jnp.zeros(qkv.shape, F32)
            h_scr[...] = jnp.zeros((TM, D), F32)
            start(cps_w(0, 1))
            wait_w(0, 0)
            cp_x(0).wait()
            start(cps_w(1, 0))
            permute_wqkv_rows(wE, 0, KC, SUB)
            for r0 in range(0, TM, LR):
                ln_chunk(xbuf[0, pl.ds(r0, LR), :], xn_scr, r0, LR)

            def mm(wsrc, m, kt):
                xt = xn_scr[kt]
                rows = pl.ds(pl.multiple_of(m * KC, KC), KC)
                for n in range(0, 3 * NT, PN):
                    rhs = jnp.concatenate([wsrc[n + jj, rows, :] for jj in range(PN)], axis=1)
                    r = jnp.dot(xt, rhs, preferred_element_type=F32)
                    for jj in range(PN):
                        qkv[n + jj, pl.ds(HALO, TM), :] += r[:, jj*128:(jj+1)*128]

            def body(m, carry):
                wait_w(m, 1)
                pl.when(m < 3)(lambda: start(cps_w(jnp.minimum(m + 1, 3), 1)))
                permute_wqkv_rows(wO, pl.multiple_of(m * KC, KC), KC, SUB)
                mm(wE, m, 2 * m)
                pl.when(m < 3)(lambda: wait_w(jnp.minimum(m + 1, 3), 0))
                pl.when(m < 2)(lambda: start(cps_w(jnp.minimum(m + 2, 3), 0)))
                @pl.when(m == 2)
                def _():
                    start(cps_tiles(wo_hbm, wo_ref, sem_o.at[0]))
                    cp_x(1).start()
                pl.when(m == 3)(lambda: start(cps_tiles(w1_hbm, w1_ref, sem_o.at[1])))
                permute_wqkv_rows(wE, pl.multiple_of((m + 1) * KC, KC), KC, SUB)
                mm(wO, m, 2 * m + 1)
                return carry
            jax.lax.fori_loop(0, 4, body, 0)

        @pl.when(i + 2 < NB)
        def _():
            cp_x(i + 2).start()

        @pl.when(i + 1 < NB)
        def _():
            cp_x(i + 1).wait()

        def ln_next(r0):
            return ln_chunk(xbuf[(i + 1) % 3, pl.ds(r0, LR), :], xn_scr, r0, LR)

        @pl.when(i == 0)
        def _():
            wait_all(wo_ref, sem_o.at[0])
            for r0 in range(0, TM, R):
                attn_chunk(i, r0, R, qkv, o_scr, TM)
            halo()
            for r0 in range(0, TM, LR):
                ln_next(r0)
            permute_wo(wo_ref, range(NT))

        @pl.when(i == 1)
        def _():
            wait_all(w1_ref, sem_o.at[1])
            if not W2BAR:
                wait_all(w2_ref, sem_o.at[2])

        @pl.when(i > 0)
        def _():
            hn = load_tiles(hn_scr)
            n1 = DFF // NC1
            n2 = D // 128 * KS2
            tasks = [("a", r0) for r0 in range(0, TM, R)] + [("l", r0) for r0 in range(0, TM, LRN)]
            nslots = n1 + n2
            pos = [c * (DFF / n1) * 8 for c in range(n1)] + [DFF * 8 + c * (DFF / KS2) for c in range(n2)]
            total = 2 * DFF * 8
            assign = [[] for _ in range(nslots + 1)]
            allowed = [s for s in range(1, nslots) if not (W2BAR and s == n1)]
            for t, task in enumerate(tasks):
                target = FRAC * total * (t + S0) / (len(tasks) - 1 + S0)
                s = min(allowed, key=lambda s: abs(pos[s] - target))
                if target > pos[-1] + 0.5 * (DFF / KS2):
                    s = nslots
                assign[s].append(task)
            def run(slot):
                deps = []
                for kind, r0 in assign[slot]:
                    if kind == "a":
                        deps.append(attn_chunk(i, r0, R, qkv, o_scr, TM))
                    else:
                        deps.append(ln_chunk(xbuf[(i + 1) % 3, pl.ds(r0, LRN), :], xn_scr, r0, LRN))
                return _or(deps)
            a_parts = []
            for c in range(n1):
                dep = run(c)
                rhs = jnp.concatenate([w1_ref[c * NC1 // 128 + jj] for jj in range(NC1 // 128)], axis=1)
                a = jnp.dot(hn, gate_r(rhs, dep, pred), preferred_element_type=F32)
                a_parts.append(jnp.maximum(a, 0.0))
            a = jnp.concatenate(a_parts, axis=1).astype(BF16)
            if W2BAR:
                pl.when(i == 1)(lambda: wait_all(w2_ref, sem_o.at[2]))
            for c in range(D // 128):
                rhs = w2_ref[c]
                for ks in range(KS2):
                    dep = run(n1 + c * KS2 + ks)
                    k0 = (ks * (28 // 4) // KS2) * 512
                    rhs = gate_r(rhs, dep, pred, k0)
                y = h_scr[:, c*128:(c+1)*128] + jnp.dot(a, rhs, preferred_element_type=F32)
                o_ref[:, c*128:(c+1)*128] = y.astype(o_ref.dtype)
            run(nslots)
            halo()

        @pl.when(i == 0)
        def _():
            start(cps_tiles(w2_hbm, w2_ref, sem_o.at[2]))

        def out_proj():
            h_scr[...] = xbuf[i % 3].astype(F32) + jnp.dot(load_tiles(o_scr), load_tiles(wo_ref), preferred_element_type=F32)

        @pl.when(i < NB - 1)
        def _():
            out_proj()
            xn = load_tiles(xn_scr)
            ncs = 3 * D // NQ
            ln_rows = list(range(0, TM, LR))
            for c in range(ncs):
                dep = None
                if Q0 <= c < Q0 + len(ln_rows):
                    r0 = ln_rows[c - Q0]
                    dep = ln_chunk(h_scr[pl.ds(r0, LR), :], hn_scr, r0, LR)
                rhs = jnp.concatenate([jnp.concatenate([(wE if kt % 2 == 0 else wO)[c * NQ // 128 + jj, pl.ds((kt // 2) * KC, KC), :] for kt in range(NT)], axis=0)
                                       for jj in range(NQ // 128)], axis=1)
                r = jnp.dot(xn, gate_r(rhs, dep, pred), preferred_element_type=F32)
                for jj in range(NQ // 128):
                    qkv[c * NQ // 128 + jj, pl.ds(HALO, TM), :] = r[:, jj*128:(jj+1)*128]

        @pl.when(i == NB - 1)
        def _():
            out_proj()
            for r0 in range(0, TM, LR):
                ln_chunk(h_scr[pl.ds(r0, LR), :], hn_scr, r0, LR)

    anyspec = pl.BlockSpec(memory_space=pl.ANY)
    out = pl.pallas_call(
        kern,
        grid=(NSTEPS or NB + 1,),
        in_specs=[anyspec] * 5,
        out_specs=pl.BlockSpec((TM, D), lambda i: (jnp.maximum(i - 1, 0), 0)),
        out_shape=jax.ShapeDtypeStruct((S, D), jnp.bfloat16),
        scratch_shapes=[pltpu.VMEM((3, TM, D), BF16), pltpu.VMEM((3 * NT, 5 * KC, 128), BF16), pltpu.VMEM((3 * NT, 4 * KC, 128), BF16),
                        pltpu.VMEM((NT, D, 128), BF16),
                        pltpu.VMEM((DFF // 128, D, 128), BF16), pltpu.VMEM((NT, DFF, 128), BF16),
                        pltpu.SemaphoreType.DMA((3,)), pltpu.SemaphoreType.DMA((8,)), pltpu.SemaphoreType.DMA((3,)),
                        pltpu.VMEM((NT, TM, 128), BF16), pltpu.VMEM((3 * NT, HALO + TM, 128), F32),
                        pltpu.VMEM((NT, TM, 128), BF16), pltpu.VMEM((TM, D), F32),
                        pltpu.VMEM((NT, TM, 128), BF16)],
        compiler_params=pltpu.CompilerParams(dimension_semantics=("arbitrary",), vmem_limit_bytes=100 * 1024 * 1024, flags=flags),
    )(x, A_wqkv, wo_p, B_w1, B_w2)
    return out.reshape(1, S, D)


@jax.jit
def pallas_sequential_preLN__sliding_local_dilated__dense_activation_relu__prompt_kernel(
    A_x, A_wqkv, A_wo, B_x, B_w1, B_w2):
    return _fused(A_x, A_wqkv, A_wo, B_x, B_w1, B_w2)
```

```python
import functools
import math

import jax
import jax.numpy as jnp
import jax.experimental.pallas as pl
import jax.experimental.pallas.tpu as pltpu

F32, BF16, U32, I32 = jnp.float32, jnp.bfloat16, jnp.uint32, jnp.int32

H, W, DIL = 32, 8, 2
TM = 256
HALO = 16
R = 16
LR = 32
LRN = 64
KC = 128
KW = KC // 2
SUB = 64
EPS = 1e-5


def _ln(x):
    m = jnp.mean(x, axis=-1, keepdims=True)
    xc = x - m
    v = jnp.mean(xc * xc, axis=-1, keepdims=True)
    return xc * jax.lax.rsqrt(v + EPS)


def _dep_of(us):
    t = us[0]
    for a in us[1:]:
        t = t | a
    r = t[0:8]
    for g in range(1, t.shape[0] // 8):
        r = r | t[g * 8:(g + 1) * 8]
    return r


def _or(deps):
    if not deps:
        return None
    r = deps[0]
    for d in deps[1:]:
        r = r | d
    return r


def _gate(rhs, dep, pred, k0=0):
    if dep is None:
        return rhs
    t = pltpu.bitcast(rhs[k0:k0 + 16, 0:128], U32)
    t = pltpu.bitcast(jnp.where(pred, t, dep), BF16)
    if rhs.shape[1] > 128:
        t = jnp.concatenate([t, rhs[k0:k0 + 16, 128:]], axis=1)
    parts = ([rhs[0:k0]] if k0 else []) + [t, rhs[k0 + 16:, :]]
    return jnp.concatenate(parts, axis=0)


def _make_kernel(S, D, DFF):
    NT = D // 128
    NB = S // TM
    DH = D // H
    scale = DH ** -0.5
    c_exp2 = scale * math.log2(math.e)
    assert NT == 8 and DH == 32 and NB >= 3 and D // KC == 8 and DFF % (4 * 128) == 0

    def attn_chunk(row0, r0, qkv, o_scr, masked):
        qs = [qkv[j, pl.ds(HALO + r0, R), :] for j in range(NT)]
        ls = []
        for w in range(W):
            s = None
            for j in range(NT):
                p = qs[j] * qkv[NT + j, pl.ds(HALO + r0 - DIL * w, R), :]
                s = p if s is None else s + p
            ls.append(s)
        lane = jax.lax.broadcasted_iota(I32, (R, 128), 1)
        ls = [s + jnp.take_along_axis(s, lane ^ 1, axis=1) for s in ls]
        ls = [s + jnp.take_along_axis(s, lane ^ 2, axis=1) for s in ls]
        if masked:
            row = jax.lax.broadcasted_iota(I32, (R, 128), 0) + (r0 + row0)
            ls = [ls[0]] + [jnp.where(row >= DIL * w, ls[w], -1e9 / scale) for w in range(1, W)]
        m = ls[0]
        for w in range(1, W):
            m = jnp.maximum(m, ls[w])
        es = [jnp.exp2((l - m) * c_exp2) for l in ls]
        den = es[0]
        for w in range(1, W):
            den = den + es[w]
        inv = 1.0 / den
        ps = [e * inv for e in es]
        outs = []
        for j in range(NT):
            o = None
            for w in range(W):
                t = qkv[2 * NT + j, pl.ds(HALO + r0 - DIL * w, R), :] * ps[w]
                o = t if o is None else o + t
            outs.append(o)
        for j in range(NT):
            o_scr[j, pl.ds(r0, R), :] = outs[j].astype(BF16)
        return _dep_of([pltpu.bitcast(o, U32) for o in outs])

    def ln_chunk(src, dst_ref, r0, nrows):
        xn = _ln(src.astype(F32))
        tiles = [xn[:, j * 128:(j + 1) * 128] for j in range(NT)]
        for j in range(NT):
            dst_ref[j, pl.ds(r0, nrows), :] = tiles[j].astype(BF16)
        return _dep_of([pltpu.bitcast(t, U32) for t in tiles])

    def load_tiles(ref):
        return jnp.concatenate([ref[j] for j in range(NT)], axis=1)

    def permute_wqkv(raw, r_src, w_u, r0w):
        lane = jax.lax.broadcasted_iota(I32, (SUB // 2, 128), 1)
        grp = (lane >> 2) & 7
        masks = [grp == b for b in range(8)]
        units = [(g, s0) for g in range(3) for s0 in range(0, KC, SUB)]

        def rot(u):
            g, s0 = u
            out = []
            for j in range(NT):
                v = pltpu.bitcast(raw[pl.ds(r_src + s0, SUB), pl.ds((g * NT + j) * 128, 128)], I32)
                out.append(pltpu.roll(v, 4 * j, 1) if j else v)
            return out

        def merge(u, rs):
            g, s0 = u
            for t in range(NT):
                o = rs[0]
                for j in range(1, NT):
                    o = jnp.where(masks[(t + j) & 7], rs[j], o)
                o = pltpu.roll(o, 128 - 4 * t, 1) if t else o
                w_u[g * NT + t, pl.ds(r0w + s0 // 2, SUB // 2), :] = o

        prev = rot(units[0])
        for n, u in enumerate(units):
            nxt = rot(units[n + 1]) if n + 1 < len(units) else None
            merge(u, prev)
            prev = nxt

    def permute_wo(wo_raw, wo_u, c):
        sub = jax.lax.broadcasted_iota(I32, (8, 128), 0)
        m4 = (sub & 4) == 0
        m2 = (sub & 2) == 0
        col = pl.ds(pl.multiple_of(c * 128, 128), 128)
        for hh in range(4):
            for t2 in range(2):
                u = [pltpu.bitcast(wo_raw[pl.ds(2 * (64 * j + 16 * hh + 8 * t2), 16), col], I32) for j in range(8)]
                for j in (0, 1, 4, 5):
                    a, b = u[j], u[j + 2]
                    u[j] = jnp.where(m4, a, pltpu.roll(b, 4, 0))
                    u[j + 2] = jnp.where(m4, pltpu.roll(a, 4, 0), b)
                for j in (0, 2, 4, 6):
                    a, b = u[j], u[j + 1]
                    u[j] = jnp.where(m2, a, pltpu.roll(b, 2, 0))
                    u[j + 1] = jnp.where(m2, pltpu.roll(a, 6, 0), b)
                for idx in range(8):
                    j2, t1, t0 = idx >> 2, (idx >> 1) & 1, idx & 1
                    t = 4 * t2 + 2 * t1 + t0
                    wo_u[c, pl.ds(64 * t + 16 * hh + 8 * j2, 8), :] = u[idx]

    def kernel(x_hbm, wqkv_hbm, wo_hbm, w1_hbm, w2_hbm, o_ref,
               xbuf, wraw, wE, wO, wo_raw, wo_u, w1_ref, w2_ref, sem_x, sem_w, sem_o,
               xn_scr, xn2_scr, qkv, qkv0, o_scr, h_scr, hn_scr):
        i = pl.program_id(0)
        pred = i < 1000

        def cp_x(b):
            return pltpu.make_async_copy(x_hbm.at[pl.ds(pl.multiple_of(b * TM, TM), TM), :],
                                         xbuf.at[b % 3], sem_x.at[b % 3])

        def cp_w(c):
            r = pl.multiple_of(c * KC, KC)
            return pltpu.make_async_copy(wqkv_hbm.at[pl.ds(r, KC), :], wraw.at[pl.ds(r, KC), :], sem_w.at[c])

        cp_wo = pltpu.make_async_copy(wo_hbm, wo_raw.at[:, pl.ds(0, D)], sem_o.at[0])
        cp_w1 = pltpu.make_async_copy(w1_hbm, w1_ref, sem_o.at[1])
        cp_w2 = pltpu.make_async_copy(w2_hbm, w2_ref, sem_o.at[2])

        def w_tile(n):
            return jnp.concatenate(
                [pltpu.bitcast((wE if kt % 2 == 0 else wO)[n, pl.ds((kt // 2) * KW, KW), :], BF16)
                 for kt in range(NT)], axis=0)

        @pl.when(i == 0)
        def _():
            for r0 in range(0, TM, 32):
                pltpu.make_async_copy(x_hbm.at[pl.ds(r0, 32), :], xbuf.at[0, pl.ds(r0, 32), :], sem_x.at[0]).start()
            cp_w(0).start()
            qkv0[...] = jnp.zeros(qkv0.shape, F32)
            cp_x(0).wait()
            cp_w(1).start()
            for r0 in range(0, TM, LR):
                ln_chunk(xbuf[0, pl.ds(r0, LR), :], xn_scr, r0, LR)
            cp_w(0).wait()
            cp_w(2).start()
            permute_wqkv(wraw, 0, wE, 0)

            def mm(wsrc, m, kt):
                xt = xn_scr[kt]
                rows = pl.ds(pl.multiple_of(m * KW, KW), KW)
                for n in range(0, 3 * NT, 2):
                    rhs = jnp.concatenate([pltpu.bitcast(wsrc[n + jj, rows, :], BF16) for jj in range(2)], axis=1)
                    r = jnp.dot(xt, rhs, preferred_element_type=F32)
                    for jj in range(2):
                        qkv0[n + jj, pl.ds(HALO, TM), :] += r[:, jj * 128:(jj + 1) * 128]

            def body(m, carry):
                def ln1_piece(c):
                    r = pl.multiple_of(64 * (c % 4), 64)
                    ln_chunk(xbuf[jnp.where(m >= 2, 1, 0), pl.ds(r, 64), :], xn2_scr, r, 64)

                cp_w(2 * m + 1).wait()
                pl.when(m == 2)(lambda: cp_x(1).wait())
                pl.when(m < 3)(lambda: cp_w(jnp.minimum(2 * m + 3, 7)).start())
                ln1_piece(2 * m)
                permute_wqkv(wraw, pl.multiple_of((2 * m + 1) * KC, KC), wO, pl.multiple_of(m * KW, KW))
                mm(wE, m, 2 * m)
                pl.when(m < 3)(lambda: cp_w(jnp.minimum(2 * m + 2, 7)).wait())
                pl.when(m < 2)(lambda: cp_w(jnp.minimum(2 * m + 4, 7)).start())
                pl.when(m == 1)(lambda: cp_x(1).start())
                pl.when(m == 2)(lambda: cp_wo.start())
                ln1_piece(2 * m + 1)
                permute_wqkv(wraw, pl.multiple_of(jnp.minimum(2 * m + 2, 7) * KC, KC), wE,
                             pl.multiple_of((m + 1) * KW, KW))
                mm(wO, m, 2 * m + 1)
                return carry

            jax.lax.fori_loop(0, D // KC // 2, body, 0)

        @pl.when(i + 2 < NB)
        def _():
            cp_x(i + 2).start()

        @pl.when((i > 0) & (i + 1 < NB))
        def _():
            cp_x(i + 1).wait()

        @pl.when(i == 0)
        def _():
            for j in range(NT, 3 * NT):
                qkv[j, pl.ds(0, HALO), :] = qkv0[j, pl.ds(TM, HALO), :]
            cp_w1.start()
            NI, R0, per = 4, TM // 4, 3
            nt = 3 * NT // NI

            def body(m, carry):
                r_base = pl.multiple_of(m * R0, R0)
                pl.when(m == 1)(lambda: cp_wo.wait())
                cols = [jnp.where(m == 0, NT + cc, jnp.minimum((m - 1) * per + cc, NT - 1)) for cc in range(per)]
                for c in cols:
                    permute_wo(wo_raw, wo_u, c)
                xn = load_tiles(xn2_scr)
                for jj in range(nt):
                    dep = None
                    if jj >= nt - R0 // R:
                        dep = attn_chunk(0, r_base + (jj - (nt - R0 // R)) * R, qkv0, o_scr, True)
                    n = m * nt + jj
                    qkv[n, pl.ds(HALO, TM), :] = jnp.dot(xn, _gate(w_tile(n), dep, pred), preferred_element_type=F32)
                return carry

            jax.lax.fori_loop(0, NI, body, 0)

        @pl.when(i == 1)
        def _():
            cp_w1.wait()

        @pl.when(i > 0)
        def _():
            hn = load_tiles(hn_scr)
            KS2 = 2
            n1, n2 = DFF // 128, NT * KS2
            tasks = [("a", r0) for r0 in range(0, TM, R)] + [("l", r0) for r0 in range(0, TM, LRN)]
            nslots = n1 + n2
            pos = [c * 128 * 8 for c in range(n1)] + [DFF * 8 + c * (DFF / KS2) for c in range(n2)]
            total = 2 * DFF * 8
            assign = [[] for _ in range(nslots + 1)]
            allowed = [s for s in range(1, nslots) if s != n1]
            for t, task in enumerate(tasks):
                target = total * (t + 1) / len(tasks)
                s = min(allowed, key=lambda s: abs(pos[s] - target))
                if target > pos[-1] + 0.5 * (DFF / KS2):
                    s = nslots
                assign[s].append(task)

            def run(slot):
                deps = []
                for kind, r0 in assign[slot]:
                    if kind == "a":
                        deps.append(attn_chunk(i * TM, r0, qkv, o_scr, r0 < DIL * (W - 1)))
                    else:
                        deps.append(ln_chunk(xbuf[(i + 1) % 3, pl.ds(r0, LRN), :], xn_scr, r0, LRN))
                return _or(deps)

            a_parts = []
            for c in range(n1):
                a = jnp.dot(hn, _gate(w1_ref[:, c * 128:(c + 1) * 128], run(c), pred), preferred_element_type=F32)
                a_parts.append(jnp.maximum(a, 0.0))
            a = jnp.concatenate(a_parts, axis=1).astype(BF16)
            pl.when(i == 1)(lambda: cp_w2.wait())
            for c in range(NT):
                rhs = w2_ref[:, c * 128:(c + 1) * 128]
                for ks in range(KS2):
                    rhs = _gate(rhs, run(n1 + c * KS2 + ks), pred, (ks * (DFF // 512) // KS2) * 512)
                y = h_scr[:, c * 128:(c + 1) * 128] + jnp.dot(a, rhs, preferred_element_type=F32)
                o_ref[:, c * 128:(c + 1) * 128] = y.astype(o_ref.dtype)
            run(nslots)
            for j in range(NT, 3 * NT):
                qkv[j, pl.ds(0, HALO), :] = qkv[j, pl.ds(TM, HALO), :]

        @pl.when(i == 0)
        def _():
            cp_w2.start()

        def out_proj():
            wo = jnp.concatenate([pltpu.bitcast(wo_u[j], BF16) for j in range(NT)], axis=1)
            h_scr[...] = xbuf[i % 3].astype(F32) + jnp.dot(load_tiles(o_scr), wo, preferred_element_type=F32)

        @pl.when((i > 0) & (i < NB - 1))
        def _():
            out_proj()
            xn = load_tiles(xn_scr)
            ln_rows = list(range(0, TM, LR))
            for c in range(3 * NT // 2):
                dep = None
                if 1 <= c <= len(ln_rows):
                    r0 = ln_rows[c - 1]
                    dep = ln_chunk(h_scr[pl.ds(r0, LR), :], hn_scr, r0, LR)
                rhs = jnp.concatenate([w_tile(2 * c), w_tile(2 * c + 1)], axis=1)
                r = jnp.dot(xn, _gate(rhs, dep, pred), preferred_element_type=F32)
                for jj in range(2):
                    qkv[2 * c + jj, pl.ds(HALO, TM), :] = r[:, jj * 128:(jj + 1) * 128]

        @pl.when((i == 0) | (i == NB - 1))
        def _():
            out_proj()
            for r0 in range(0, TM, LR):
                ln_chunk(h_scr[pl.ds(r0, LR), :], hn_scr, r0, LR)

    scratch = [
        pltpu.VMEM((3, TM, D), BF16),
        pltpu.VMEM((D, 3 * D), BF16),
        pltpu.VMEM((3 * NT, 5 * KW, 128), I32),
        pltpu.VMEM((3 * NT, 4 * KW, 128), I32),
        pltpu.VMEM((D, D + 384), BF16),
        pltpu.VMEM((NT + 3, D // 2, 128), I32),
        pltpu.VMEM((D, DFF), BF16),
        pltpu.VMEM((DFF, D), BF16),
        pltpu.SemaphoreType.DMA((3,)),
        pltpu.SemaphoreType.DMA((D // KC,)),
        pltpu.SemaphoreType.DMA((3,)),
        pltpu.VMEM((NT, TM, 128), BF16),
        pltpu.VMEM((NT, TM, 128), BF16),
        pltpu.VMEM((3 * NT, HALO + TM, 128), F32),
        pltpu.VMEM((3 * NT, HALO + TM, 128), F32),
        pltpu.VMEM((NT, TM, 128), BF16),
        pltpu.VMEM((TM, D), F32),
        pltpu.VMEM((NT, TM, 128), BF16),
    ]
    return kernel, scratch, NB


@jax.jit
def pallas_sequential_preLN__sliding_local_dilated__dense_activation_relu__prompt_kernel(
    A_x: jax.Array,
    A_wqkv: jax.Array,
    A_wo: jax.Array,
    B_x: jax.Array,
    B_w1: jax.Array,
    B_w2: jax.Array,
):
    del B_x
    B, S, D = A_x.shape
    DFF = B_w1.shape[1]
    assert B == 1
    kernel, scratch, NB = _make_kernel(S, D, DFF)
    hbm = pl.BlockSpec(memory_space=pl.ANY)
    out = pl.pallas_call(
        kernel,
        grid=(NB + 1,),
        in_specs=[hbm] * 5,
        out_specs=pl.BlockSpec((TM, D), lambda i: (jnp.maximum(i - 1, 0), 0)),
        out_shape=jax.ShapeDtypeStruct((S, D), A_x.dtype),
        scratch_shapes=scratch,
        compiler_params=pltpu.CompilerParams(dimension_semantics=("arbitrary",),
                                             vmem_limit_bytes=100 * 1024 * 1024),
    )(A_x.reshape(S, D), A_wqkv, A_wo, B_w1, B_w2)
    return out.reshape(B, S, D)
```

```python
import functools
import math

import jax
import jax.numpy as jnp
import jax.experimental.pallas as pl
import jax.experimental.pallas.tpu as pltpu

F32, BF16, U32, I32 = jnp.float32, jnp.bfloat16, jnp.uint32, jnp.int32

H, W, DIL = 32, 8, 2
TM = 256
HALO = 16
R = 16
LR = 32
LRN = 64
KC = 128
KW = KC // 2
SUB = 64
EPS = 1e-5


def _ln(x):
    m = jnp.mean(x, axis=-1, keepdims=True)
    xc = x - m
    v = jnp.mean(xc * xc, axis=-1, keepdims=True)
    return xc * jax.lax.rsqrt(v + EPS)


def _dep_of(us):
    t = us[0]
    for a in us[1:]:
        t = t | a
    r = t[0:8]
    for g in range(1, t.shape[0] // 8):
        r = r | t[g * 8:(g + 1) * 8]
    return r


def _or(deps):
    if not deps:
        return None
    r = deps[0]
    for d in deps[1:]:
        r = r | d
    return r


def _gate(rhs, dep, pred, k0=0):
    if dep is None:
        return rhs
    t = pltpu.bitcast(rhs[k0:k0 + 16, 0:128], U32)
    t = pltpu.bitcast(jnp.where(pred, t, dep), BF16)
    if rhs.shape[1] > 128:
        t = jnp.concatenate([t, rhs[k0:k0 + 16, 128:]], axis=1)
    parts = ([rhs[0:k0]] if k0 else []) + [t, rhs[k0 + 16:, :]]
    return jnp.concatenate(parts, axis=0)


def _make_kernel(S, D, DFF):
    NT = D // 128
    NB = S // TM
    DH = D // H
    scale = DH ** -0.5
    c_exp2 = scale * math.log2(math.e)
    assert NT == 8 and DH == 32 and NB >= 3 and D // KC == 8 and DFF % (4 * 128) == 0

    def attn_chunk(row0, r0, qkv, o_scr, masked):
        qs = [qkv[j, pl.ds(HALO + r0, R), :] for j in range(NT)]
        ls = []
        for w in range(W):
            s = None
            for j in range(NT):
                p = qs[j] * qkv[NT + j, pl.ds(HALO + r0 - DIL * w, R), :]
                s = p if s is None else s + p
            ls.append(s)
        lane = jax.lax.broadcasted_iota(I32, (R, 128), 1)
        ls = [s + jnp.take_along_axis(s, lane ^ 1, axis=1) for s in ls]
        ls = [s + jnp.take_along_axis(s, lane ^ 2, axis=1) for s in ls]
        if masked:
            row = jax.lax.broadcasted_iota(I32, (R, 128), 0) + (r0 + row0)
            ls = [ls[0]] + [jnp.where(row >= DIL * w, ls[w], -1e9 / scale) for w in range(1, W)]
        m = ls[0]
        for w in range(1, W):
            m = jnp.maximum(m, ls[w])
        es = [jnp.exp2((l - m) * c_exp2) for l in ls]
        den = es[0]
        for w in range(1, W):
            den = den + es[w]
        inv = 1.0 / den
        ps = [e * inv for e in es]
        outs = []
        for j in range(NT):
            o = None
            for w in range(W):
                t = qkv[2 * NT + j, pl.ds(HALO + r0 - DIL * w, R), :] * ps[w]
                o = t if o is None else o + t
            outs.append(o)
        for j in range(NT):
            o_scr[j, pl.ds(r0, R), :] = outs[j].astype(BF16)
        return _dep_of([pltpu.bitcast(o, U32) for o in outs])

    def ln_chunk(src, dst_ref, r0, nrows):
        xn = _ln(src.astype(F32))
        tiles = [xn[:, j * 128:(j + 1) * 128] for j in range(NT)]
        for j in range(NT):
            dst_ref[j, pl.ds(r0, nrows), :] = tiles[j].astype(BF16)
        return _dep_of([pltpu.bitcast(t, U32) for t in tiles])

    def load_tiles(ref):
        return jnp.concatenate([ref[j] for j in range(NT)], axis=1)

    def permute_wqkv(raw, r_src, w_u, r0w):
        lane = jax.lax.broadcasted_iota(I32, (SUB // 2, 128), 1)
        grp = (lane >> 2) & 7
        masks = [grp == b for b in range(8)]
        units = [(g, s0) for g in range(3) for s0 in range(0, KC, SUB)]

        def rot(u):
            g, s0 = u
            out = []
            for j in range(NT):
                v = pltpu.bitcast(raw[pl.ds(r_src + s0, SUB), pl.ds((g * NT + j) * 128, 128)], I32)
                out.append(pltpu.roll(v, 4 * j, 1) if j else v)
            return out

        def merge(u, rs):
            g, s0 = u
            for t in range(NT):
                o = rs[0]
                for j in range(1, NT):
                    o = jnp.where(masks[(t + j) & 7], rs[j], o)
                o = pltpu.roll(o, 128 - 4 * t, 1) if t else o
                w_u[g * NT + t, pl.ds(r0w + s0 // 2, SUB // 2), :] = o

        prev = rot(units[0])
        for n, u in enumerate(units):
            nxt = rot(units[n + 1]) if n + 1 < len(units) else None
            merge(u, prev)
            prev = nxt

    def permute_wo(wo_raw, wo_u, c):
        sub = jax.lax.broadcasted_iota(I32, (8, 128), 0)
        m4 = (sub & 4) == 0
        m2 = (sub & 2) == 0
        col = pl.ds(pl.multiple_of(c * 128, 128), 128)
        for hh in range(4):
            for t2 in range(2):
                u = [pltpu.bitcast(wo_raw[pl.ds(2 * (64 * j + 16 * hh + 8 * t2), 16), col], I32) for j in range(8)]
                for j in (0, 1, 4, 5):
                    a, b = u[j], u[j + 2]
                    u[j] = jnp.where(m4, a, pltpu.roll(b, 4, 0))
                    u[j + 2] = jnp.where(m4, pltpu.roll(a, 4, 0), b)
                for j in (0, 2, 4, 6):
                    a, b = u[j], u[j + 1]
                    u[j] = jnp.where(m2, a, pltpu.roll(b, 2, 0))
                    u[j + 1] = jnp.where(m2, pltpu.roll(a, 6, 0), b)
                for idx in range(8):
                    j2, t1, t0 = idx >> 2, (idx >> 1) & 1, idx & 1
                    t = 4 * t2 + 2 * t1 + t0
                    wo_u[c, pl.ds(64 * t + 16 * hh + 8 * j2, 8), :] = u[idx]

    def kernel(x_hbm, wqkv_hbm, wo_hbm, w1_hbm, w2_hbm, o_ref,
               xbuf, wraw, wE, wO, wo_raw, wo_u, w1_ref, w2_ref, sem_x, sem_w, sem_o,
               xn_scr, xn2_scr, qkv, qkv0, o_scr, h_scr, hn_scr):
        i = pl.program_id(0)
        pred = i < 1000

        def cp_x(b):
            return pltpu.make_async_copy(x_hbm.at[pl.ds(pl.multiple_of(b * TM, TM), TM), :],
                                         xbuf.at[b % 3], sem_x.at[b % 3])

        def cp_w(c):
            r = pl.multiple_of(c * KC, KC)
            return pltpu.make_async_copy(wqkv_hbm.at[pl.ds(r, KC), :], wraw.at[pl.ds(r, KC), :], sem_w.at[c])

        cp_wo = pltpu.make_async_copy(wo_hbm, wo_raw.at[:, pl.ds(0, D)], sem_o.at[0])
        cp_w1 = pltpu.make_async_copy(w1_hbm.bitcast(I32), w1_ref, sem_o.at[1])
        cp_w2 = pltpu.make_async_copy(w2_hbm.bitcast(I32), w2_ref, sem_o.at[2])

        def w_tile(n):
            return jnp.concatenate(
                [pltpu.bitcast((wE if kt % 2 == 0 else wO)[n, pl.ds((kt // 2) * KW, KW), :], BF16)
                 for kt in range(NT)], axis=0)

        @pl.when(i == 0)
        def _():
            for r0 in range(0, TM, 32):
                pltpu.make_async_copy(x_hbm.at[pl.ds(r0, 32), :], xbuf.at[0, pl.ds(r0, 32), :], sem_x.at[0]).start()
            cp_w(0).start()
            qkv0[...] = jnp.zeros(qkv0.shape, F32)
            cp_x(0).wait()
            cp_w(1).start()
            for r0 in range(0, TM, LR):
                ln_chunk(xbuf[0, pl.ds(r0, LR), :], xn_scr, r0, LR)
            cp_w(0).wait()
            cp_w(2).start()
            permute_wqkv(wraw, 0, wE, 0)

            def mm(wsrc, m, kt):
                xt = xn_scr[kt]
                rows = pl.ds(pl.multiple_of(m * KW, KW), KW)
                for n in range(0, 3 * NT, 2):
                    rhs = jnp.concatenate([pltpu.bitcast(wsrc[n + jj, rows, :], BF16) for jj in range(2)], axis=1)
                    r = jnp.dot(xt, rhs, preferred_element_type=F32)
                    for jj in range(2):
                        qkv0[n + jj, pl.ds(HALO, TM), :] += r[:, jj * 128:(jj + 1) * 128]

            def body(m, carry):
                def ln1_piece(c):
                    r = pl.multiple_of(64 * (c % 4), 64)
                    ln_chunk(xbuf[jnp.where(m >= 2, 1, 0), pl.ds(r, 64), :], xn2_scr, r, 64)

                cp_w(2 * m + 1).wait()
                pl.when(m == 2)(lambda: cp_x(1).wait())
                pl.when(m < 3)(lambda: cp_w(jnp.minimum(2 * m + 3, 7)).start())
                ln1_piece(2 * m)
                permute_wqkv(wraw, pl.multiple_of((2 * m + 1) * KC, KC), wO, pl.multiple_of(m * KW, KW))
                mm(wE, m, 2 * m)
                pl.when(m < 3)(lambda: cp_w(jnp.minimum(2 * m + 2, 7)).wait())
                pl.when(m < 2)(lambda: cp_w(jnp.minimum(2 * m + 4, 7)).start())
                pl.when(m == 1)(lambda: cp_x(1).start())
                pl.when(m == 2)(lambda: cp_wo.start())
                ln1_piece(2 * m + 1)
                permute_wqkv(wraw, pl.multiple_of(jnp.minimum(2 * m + 2, 7) * KC, KC), wE,
                             pl.multiple_of((m + 1) * KW, KW))
                mm(wO, m, 2 * m + 1)
                return carry

            jax.lax.fori_loop(0, D // KC // 2, body, 0)

        @pl.when(i + 2 < NB)
        def _():
            cp_x(i + 2).start()

        @pl.when((i > 0) & (i + 1 < NB))
        def _():
            cp_x(i + 1).wait()

        @pl.when(i == 0)
        def _():
            for j in range(NT, 3 * NT):
                qkv[j, pl.ds(0, HALO), :] = qkv0[j, pl.ds(TM, HALO), :]
            cp_w1.start()
            NI, R0, per = 4, TM // 4, 3
            nt = 3 * NT // NI

            def body(m, carry):
                r_base = pl.multiple_of(m * R0, R0)
                pl.when(m == 1)(lambda: cp_wo.wait())
                cols = [jnp.where(m == 0, NT + cc, jnp.minimum((m - 1) * per + cc, NT - 1)) for cc in range(per)]
                for c in cols:
                    permute_wo(wo_raw, wo_u, c)
                xn = load_tiles(xn2_scr)
                for jj in range(nt):
                    dep = None
                    if jj >= nt - R0 // R:
                        dep = attn_chunk(0, r_base + (jj - (nt - R0 // R)) * R, qkv0, o_scr, True)
                    n = m * nt + jj
                    qkv[n, pl.ds(HALO, TM), :] = jnp.dot(xn, _gate(w_tile(n), dep, pred), preferred_element_type=F32)
                return carry

            jax.lax.fori_loop(0, NI, body, 0)

        @pl.when(i == 1)
        def _():
            cp_w1.wait()

        @pl.when(i > 0)
        def _():
            hn = load_tiles(hn_scr)
            KS2 = 2
            n1, n2 = DFF // 128, NT * KS2
            tasks = [("a", r0) for r0 in range(0, TM, R)] + [("l", r0) for r0 in range(0, TM, LRN)]
            nslots = n1 + n2
            pos = [c * 128 * 8 for c in range(n1)] + [DFF * 8 + c * (DFF / KS2) for c in range(n2)]
            total = 2 * DFF * 8
            assign = [[] for _ in range(nslots + 1)]
            allowed = [s for s in range(1, nslots) if s != n1]
            for t, task in enumerate(tasks):
                target = total * (t + 1) / len(tasks)
                s = min(allowed, key=lambda s: abs(pos[s] - target))
                if target > pos[-1] + 0.5 * (DFF / KS2):
                    s = nslots
                assign[s].append(task)

            def run(slot):
                deps = []
                for kind, r0 in assign[slot]:
                    if kind == "a":
                        deps.append(attn_chunk(i * TM, r0, qkv, o_scr, r0 < DIL * (W - 1)))
                    else:
                        deps.append(ln_chunk(xbuf[(i + 1) % 3, pl.ds(r0, LRN), :], xn_scr, r0, LRN))
                return _or(deps)

            a_parts = []
            for c in range(n1):
                a = jnp.dot(hn, _gate(pltpu.bitcast(w1_ref[:, c * 128:(c + 1) * 128], BF16), run(c), pred), preferred_element_type=F32)
                a_parts.append(jnp.maximum(a, 0.0))
            a = jnp.concatenate(a_parts, axis=1).astype(BF16)
            pl.when(i == 1)(lambda: cp_w2.wait())
            for c in range(NT):
                rhs = pltpu.bitcast(w2_ref[:, c * 128:(c + 1) * 128], BF16)
                for ks in range(KS2):
                    rhs = _gate(rhs, run(n1 + c * KS2 + ks), pred, (ks * (DFF // 512) // KS2) * 512)
                y = h_scr[:, c * 128:(c + 1) * 128] + jnp.dot(a, rhs, preferred_element_type=F32)
                o_ref[:, c * 128:(c + 1) * 128] = y.astype(o_ref.dtype)
            run(nslots)
            for j in range(NT, 3 * NT):
                qkv[j, pl.ds(0, HALO), :] = qkv[j, pl.ds(TM, HALO), :]

        @pl.when(i == 0)
        def _():
            cp_w2.start()

        def out_proj():
            wo = jnp.concatenate([pltpu.bitcast(wo_u[j], BF16) for j in range(NT)], axis=1)
            h_scr[...] = xbuf[i % 3].astype(F32) + jnp.dot(load_tiles(o_scr), wo, preferred_element_type=F32)

        @pl.when((i > 0) & (i < NB - 1))
        def _():
            out_proj()
            xn = load_tiles(xn_scr)
            ln_rows = list(range(0, TM, LR))
            for c in range(3 * NT // 2):
                dep = None
                if 1 <= c <= len(ln_rows):
                    r0 = ln_rows[c - 1]
                    dep = ln_chunk(h_scr[pl.ds(r0, LR), :], hn_scr, r0, LR)
                rhs = jnp.concatenate([w_tile(2 * c), w_tile(2 * c + 1)], axis=1)
                r = jnp.dot(xn, _gate(rhs, dep, pred), preferred_element_type=F32)
                for jj in range(2):
                    qkv[2 * c + jj, pl.ds(HALO, TM), :] = r[:, jj * 128:(jj + 1) * 128]

        @pl.when((i == 0) | (i == NB - 1))
        def _():
            out_proj()
            for r0 in range(0, TM, LR):
                ln_chunk(h_scr[pl.ds(r0, LR), :], hn_scr, r0, LR)

    scratch = [
        pltpu.VMEM((3, TM, D), BF16),
        pltpu.VMEM((D, 3 * D), BF16),
        pltpu.VMEM((3 * NT, 5 * KW, 128), I32),
        pltpu.VMEM((3 * NT, 4 * KW, 128), I32),
        pltpu.VMEM((D, D + 384), BF16),
        pltpu.VMEM((NT + 3, D // 2, 128), I32),
        pltpu.VMEM((D // 2, DFF), I32),
        pltpu.VMEM((DFF // 2, D), I32),
        pltpu.SemaphoreType.DMA((3,)),
        pltpu.SemaphoreType.DMA((D // KC,)),
        pltpu.SemaphoreType.DMA((3,)),
        pltpu.VMEM((NT, TM, 128), BF16),
        pltpu.VMEM((NT, TM, 128), BF16),
        pltpu.VMEM((3 * NT, HALO + TM, 128), F32),
        pltpu.VMEM((3 * NT, HALO + TM, 128), F32),
        pltpu.VMEM((NT, TM, 128), BF16),
        pltpu.VMEM((TM, D), F32),
        pltpu.VMEM((NT, TM, 128), BF16),
    ]
    return kernel, scratch, NB


@jax.jit
def pallas_sequential_preLN__sliding_local_dilated__dense_activation_relu__prompt_kernel(
    A_x: jax.Array,
    A_wqkv: jax.Array,
    A_wo: jax.Array,
    B_x: jax.Array,
    B_w1: jax.Array,
    B_w2: jax.Array,
):
    del B_x
    B, S, D = A_x.shape
    DFF = B_w1.shape[1]
    assert B == 1
    kernel, scratch, NB = _make_kernel(S, D, DFF)
    hbm = pl.BlockSpec(memory_space=pl.ANY)
    out = pl.pallas_call(
        kernel,
        grid=(NB + 1,),
        in_specs=[hbm] * 5,
        out_specs=pl.BlockSpec((TM, D), lambda i: (jnp.maximum(i - 1, 0), 0)),
        out_shape=jax.ShapeDtypeStruct((S, D), A_x.dtype),
        scratch_shapes=scratch,
        compiler_params=pltpu.CompilerParams(dimension_semantics=("arbitrary",),
                                             vmem_limit_bytes=100 * 1024 * 1024),
    )(A_x.reshape(S, D), A_wqkv, A_wo, B_w1, B_w2)
    return out.reshape(B, S, D)
```
